```python
import os as _os
_os.environ.setdefault("JAX_PLATFORMS", "cpu")
import jax
import jax.numpy as jnp

def _softmax(x, axis=-1):
    return jax.nn.softmax(x, axis=axis)
def _gelu(x):
    return jax.nn.gelu(x, approximate=True)
def _silu(x):
    return jax.nn.silu(x)
def _sigmoid(x):
    return jax.nn.sigmoid(x)
def _layernorm(x, axis=-1, eps=1e-5):
    m = jnp.mean(x, axis=axis, keepdims=True)
    v = jnp.var(x, axis=axis, keepdims=True)
    return (x - m) / jnp.sqrt(v + eps)
def _scatter_add(tgt, idx, src, axis=0):
    return tgt.at[idx].add(src)
def _segment_sum(src, seg, n):
    return jax.ops.segment_sum(src, seg, n)
class _Rng:
    def __init__(self, key):
        self._k = key
    def _next(self):
        self._k, sub = jax.random.split(self._k)
        return sub
    def normal(self, shape):
        return jax.random.normal(self._next(), shape, dtype=jnp.bfloat16)
    def randint(self, lo, hi, shape):
        return jax.random.randint(self._next(), shape, lo, hi, dtype=jnp.int32)
    def uniform(self, shape, lo=0.0, hi=1.0):
        return jax.random.uniform(self._next(), shape, jnp.bfloat16, lo, hi)
    def permutation(self, n):
        return jax.random.permutation(self._next(), n)


kernel_name = 'standalone__gqa_block_cached__near_ridge'

def setup_inputs():
    _rng = _Rng(jax.random.key(int.from_bytes(__import__("os").urandom(4), "little")))
    _w = (lambda a: (lambda t: t.astype(jnp.bfloat16) if jnp.issubdtype(t.dtype, jnp.floating) else t)(jnp.asarray(a)))
    B, Sq, D = 8, 96, 448
    Hq, Hkv, Sk, Dh = 16, 8, 2048, 256
    assert Hq % Hkv == 0, (Hq, Hkv)
    return {
        "x": _w((lambda *s: _rng.normal(s) * 0.8)(B, Sq, D)),
        "k_cache": _w((lambda *s: _rng.normal(s) * 0.8)(B, Hkv, Sk, Dh)),
        "v_cache": _w((lambda *s: _rng.normal(s) * 0.05)(B, Hkv, Sk, Dh)),
        "wq": _w((lambda *s: _rng.normal(s) * 0.8)(D, Hq * Dh) * (D ** -0.5)),
        "wo": _w((lambda *s: _rng.normal(s) * 0.05)(Hq * Dh, D) * ((Hq * Dh) ** -0.5)),
    }

def reference(x, k_cache, v_cache, wq, wo):
    B, Sq, D = x.shape
    Hq, Dh = 16, 256
    Hkv = k_cache.shape[1]
    rep = Hq // Hkv
    q = (lambda x, *d: x.transpose(*d))((x @ wq).reshape(B, Sq, Hq, Dh), 0, 2, 1, 3)
    k = jnp.repeat(k_cache, rep, axis=1)
    v = jnp.repeat(v_cache, rep, axis=1)
    scores = jnp.einsum("bhqd,bhkd->bhqk", q, k) * (Dh ** -0.5)
    p = _softmax(scores, axis=-1)
    o = jnp.einsum("bhqk,bhkd->bhqd", p, v)
    return (lambda x, *d: x.transpose(*d))(o, 0, 2, 1, 3).reshape(B, Sq, Hq * Dh) @ wo
```

```python
import functools
import jax, jax.numpy as jnp
from jax import lax
import jax.experimental.pallas as pl
import jax.experimental.pallas.tpu as pltpu

LOG2E = 1.4426950408889634
NT = (((1,), (1,)), ((), ()))
f32, bf16 = jnp.float32, jnp.bfloat16

def kernel(x_hbm, k_hbm, v_hbm, wq_hbm, wot_hbm, out_hbm,
           x_sc, wq_sc, wo_sc, kbuf, vbuf, q_all, o0, o1, acc_sc, s0, s1, m0, m1, p0, p1, l0, l1, osc, out_sc,
           sem_k, sem_v, sem_w, sem_o,
           *, B, Sq, Dh, rep, Hkv, Sk, NB):
    N = B * Hkv
    G = rep * Dh
    R = rep * Sq
    G2 = R // 16
    NC = Sk // 128
    os_, ss, ms, ps, ls = (o0, o1), (s0, s1), (m0, m1), (p0, p1), (l0, l1)

    def k_copy(i):
        return pltpu.make_async_copy(k_hbm.at[i % B, i // B], kbuf.at[i % NB], sem_k.at[i % NB])

    def v_copy(i):
        return pltpu.make_async_copy(v_hbm.at[i % B, i // B], vbuf.at[i % NB], sem_v.at[i % NB])

    x_copy = pltpu.make_async_copy(x_hbm, x_sc, sem_w.at[0])
    wq_copy = pltpu.make_async_copy(wq_hbm, wq_sc, sem_w.at[1])
    wo_copy = pltpu.make_async_copy(wot_hbm, wo_sc, sem_w.at[2])

    def out_copy(b):
        return pltpu.make_async_copy(out_sc.at[b], out_hbm.at[b], sem_o.at[b])

    def outproj(i, o_src):
        h = i // B
        b = i % B
        part = acc_sc[b]
        for r in range(rep):
            col = pl.multiple_of(h * G + r * Dh, Dh)
            part = part + lax.dot_general(o_src[r * Sq:(r + 1) * Sq, :], wo_sc[:, pl.ds(col, Dh)], NT,
                                          preferred_element_type=f32)
        acc_sc[b] = part

    def pv(i, par):
        o = jnp.dot(pltpu.bitcast(ps[par][...], bf16), vbuf[i % NB], preferred_element_type=f32)
        linv = 1.0 / ls[par][...]
        for c in range(Dh // 128):
            osc[c] = o[:, c * 128:(c + 1) * 128]
        for c in range(Dh // 128):
            ev = osc[c, pl.ds(0, R // 2, stride=2), :].reshape(G2, 1, 8, 128)
            od = osc[c, pl.ds(1, R // 2, stride=2), :].reshape(G2, 1, 8, 128)
            on = jnp.concatenate([ev, od], axis=1).reshape(R, 128)
            os_[par][:, c * 128:(c + 1) * 128] = (on * linv).astype(bf16)

    def qk_exp(iq, parq, do_qk, do_exp):
        pe = 1 - parq
        if do_qk:
            sn = lax.dot_general(q_all[iq], kbuf[iq % NB], NT, preferred_element_type=f32)
            ss[parq][...] = sn
        if do_exp:
            mb = ms[pe][...]
        if do_qk:
            ms[parq][...] = jnp.broadcast_to(jnp.max(sn, axis=1, keepdims=True), (R, 128))
        if do_exp:
            lacc = jnp.zeros((R, 128), f32)
            for c in range(NC):
                xx = ss[pe][:, c * 128:(c + 1) * 128] - mb
                if do_qk:
                    xx = jnp.minimum(xx, jnp.abs(sn[:, c * 128:(c + 1) * 128]))
                p = jnp.exp2(xx)
                lacc = lacc + p
                p4 = p.reshape(G2, 2, 8, 128)
                ps[pe][:, c * 128:(c + 1) * 128] = pltpu.pack_elementwise(
                    [p4[:, 0], p4[:, 1]], packed_dtype=bf16).reshape(R // 2, 128)
            ls[pe][...] = jnp.broadcast_to(jnp.sum(lacc, axis=1, keepdims=True), (R, 128))

    def write_out(b):
        out_sc[b] = acc_sc[b].astype(out_sc.dtype)
        out_copy(b).start()

    x_copy.start()
    wq_copy.start()
    acc_sc[...] = jnp.zeros_like(acc_sc)
    o1[...] = jnp.zeros_like(o1)
    x_copy.wait()
    k_copy(0).start()
    k_copy(1).start()
    k_copy(2).start()
    v_copy(0).start()
    wo_copy.start()
    for j in range(3, NB):
        k_copy(j).start()
        v_copy(j - 2).start()
    for j in range(NB - 2, NB):
        v_copy(j).start()
    wq_copy.wait()

    def qbody(h, carry):
        xa = x_sc[...].reshape(B * Sq, x_sc.shape[-1])
        col = pl.multiple_of(h * G, G)
        q = jnp.dot(xa, wq_sc[:, pl.ds(col, G)], preferred_element_type=f32)
        q = (q * (Dh ** -0.5 * LOG2E)).astype(bf16)
        for b in range(B):
            for r in range(rep):
                q_all[h * B + b, r * Sq:(r + 1) * Sq, :] = q[b * Sq:(b + 1) * Sq, r * Dh:(r + 1) * Dh]
        return carry
    lax.fori_loop(0, Hkv, qbody, 0)

    k_copy(0).wait()
    qk_exp(0, 0, True, False)
    k_copy(NB).start()
    k_copy(1).wait()
    qk_exp(1, 1, True, True)
    k_copy(NB + 1).start()
    wo_copy.wait()

    def full(i, par):
        pv(i - 1, 1 - par)
        qk_exp(i + 1, 1 - par, True, True)
        outproj(jnp.maximum(i - 2, 0), os_[par])

    def body(i, carry):
        k_copy(i + 1).wait()
        v_copy(i - 1).wait()

        @pl.when(i % 2 == 0)
        def _():
            full(i, 0)

        @pl.when(i % 2 == 1)
        def _():
            full(i, 1)

        @pl.when(i + 1 + NB < N)
        def _():
            k_copy(i + 1 + NB).start()

        @pl.when(i - 1 + NB < N)
        def _():
            v_copy(i - 1 + NB).start()

        @pl.when(i - 2 >= N - B)
        def _():
            write_out(i - 2 - (N - B))
        return carry

    lax.fori_loop(1, N - 1, body, 0)

    i = N - 1
    v_copy(i - 1).wait()
    pv(i - 1, (i - 1) % 2)
    qk_exp(i + 1, (i + 1) % 2, False, True)
    outproj(i - 2, os_[i % 2])
    write_out(B - 3)
    v_copy(i).wait()
    pv(i, i % 2)
    outproj(i - 1, os_[(i - 1) % 2])
    write_out(B - 2)
    outproj(i, os_[i % 2])
    write_out(B - 1)
    for b in range(B):
        out_copy(b).wait()


@jax.jit
def pallas_standalone__gqa_block_cached__near_ridge_kernel(
    x: jax.Array,
    k_cache: jax.Array,
    v_cache: jax.Array,
    wq: jax.Array,
    wo: jax.Array,
):
    NB = 6
    B, Sq, D = x.shape
    _, Hkv, Sk, Dh = k_cache.shape
    Hq = wq.shape[1] // Dh
    rep = Hq // Hkv
    R = rep * Sq
    kern = functools.partial(kernel, B=B, Sq=Sq, Dh=Dh, rep=rep, Hkv=Hkv, Sk=Sk, NB=NB)
    anyspec = pl.BlockSpec(memory_space=pl.ANY)
    return pl.pallas_call(
        kern,
        in_specs=[anyspec] * 5,
        out_specs=anyspec,
        out_shape=jax.ShapeDtypeStruct((B, Sq, D), x.dtype),
        scratch_shapes=[
            pltpu.VMEM((B, Sq, D), bf16),
            pltpu.VMEM((D, Hq * Dh), bf16),
            pltpu.VMEM((D, Hq * Dh), bf16),
            pltpu.VMEM((NB, Sk, Dh), bf16),
            pltpu.VMEM((NB, Sk, Dh), bf16),
            pltpu.VMEM((B * Hkv, R, Dh), bf16),
        ] + [pltpu.VMEM((R, Dh), bf16)] * 2 + [pltpu.VMEM((B, Sq, D), f32)] +
        [pltpu.VMEM((R, Sk), f32)] * 2 + [pltpu.VMEM((R, 128), f32)] * 2 +
        [pltpu.VMEM((R // 2, Sk), jnp.uint32)] * 2 + [pltpu.VMEM((R, 128), f32)] * 2 +
        [pltpu.VMEM((Dh // 128, R, 128), f32), pltpu.VMEM((B, Sq, D), x.dtype)] + [
            pltpu.SemaphoreType.DMA((NB,)),
            pltpu.SemaphoreType.DMA((NB,)),
            pltpu.SemaphoreType.DMA((3,)),
            pltpu.SemaphoreType.DMA((B,)),
        ],
        compiler_params=pltpu.CompilerParams(vmem_limit_bytes=100 * 1024 * 1024, disable_bounds_checks=True),
    )(x, k_cache, v_cache, wq, wo.T)
```

```python
import functools

import jax
import jax.numpy as jnp
from jax import lax
import jax.experimental.pallas as pl
import jax.experimental.pallas.tpu as pltpu

_LOG2E = 1.4426950408889634
_NT = (((1,), (1,)), ((), ()))
_f32, _bf16 = jnp.float32, jnp.bfloat16


def _kernel(x_hbm, k_hbm, v_hbm, wq_hbm, wot_hbm, out_hbm,
            x_sc, wq_sc, wo_sc, kbuf, vbuf, q_all, o_sc, acc_sc,
            s0, s1, m0, m1, p0, p1, l0, l1,
            osc, opart, mtmp, ltmp, out_sc,
            sem_k, sem_v, sem_w, sem_q, sem_o,
            *, B, Sq, Dh, rep, Hkv, Sk, NB, E):
    N = B * Hkv
    G = rep * Dh
    R = rep * Sq
    G2 = R // 16
    NC = Sk // 128
    HS = Sk // 2
    LB = B.bit_length() - 1
    ss, ms, ps, ls = (s0, s1), (m0, m1), (p0, p1), (l0, l1)

    def slot(i):
        return i % NB if isinstance(i, int) else lax.rem(i, NB)

    def bidx(i):
        return i % B if isinstance(i, int) else jnp.bitwise_and(i, B - 1)

    def hidx(i):
        return i // B if isinstance(i, int) else lax.shift_right_logical(i, LB)

    def kv_copy(hbm, buf, sem, i, hf):
        if hf is None:
            return pltpu.make_async_copy(hbm.at[bidx(i), hidx(i)], buf.at[slot(i)], sem.at[0, slot(i)])
        return pltpu.make_async_copy(hbm.at[bidx(i), hidx(i), pl.ds(hf * HS, HS)],
                                     buf.at[slot(i), pl.ds(hf * HS, HS)], sem.at[hf, slot(i)])

    def k_copy(i, hf=None):
        return kv_copy(k_hbm, kbuf, sem_k, i, hf)

    def v_copy(i, hf=None):
        return kv_copy(v_hbm, vbuf, sem_v, i, hf)

    x_copy = pltpu.make_async_copy(x_hbm, x_sc, sem_w.at[0])
    wo_copy = pltpu.make_async_copy(wot_hbm, wo_sc, sem_w.at[1])

    def wq_copy(h):
        col = h * G if isinstance(h, int) else pl.multiple_of(h * G, G)
        return pltpu.make_async_copy(wq_hbm.at[:, pl.ds(col, G)], wq_sc.at[h], sem_q.at[h])

    def out_copy(b):
        return pltpu.make_async_copy(out_sc.at[b], out_hbm.at[b], sem_o.at[b])

    def outproj(i):
        h = hidx(i)
        b = bidx(i)
        part = acc_sc[b]
        for r in range(rep):
            col = pl.multiple_of(h * G + r * Dh, Dh)
            part = part + lax.dot_general(o_sc[r * Sq:(r + 1) * Sq, :], wo_sc[:, pl.ds(col, Dh)], _NT,
                                          preferred_element_type=_f32)
        acc_sc[b] = part

    def exp_chunk(pe, mb, c, lacc, pace):
        xx = ss[pe][:, c * 128:(c + 1) * 128] - mb
        xx = jnp.minimum(xx, jnp.abs(pace))
        p = jnp.exp2(xx)
        p4 = p.reshape(G2, 2, 8, 128)
        ps[pe][:, c * 128:(c + 1) * 128] = pltpu.pack_elementwise(
            [p4[:, 0], p4[:, 1]], packed_dtype=_bf16).reshape(R // 2, 128)
        return lacc + p

    def finish_o(o, par):
        linv = 1.0 / ls[par][...]
        for c in range(Dh // 128):
            osc[c] = o[:, c * 128:(c + 1) * 128]
        for c in range(Dh // 128):
            ev = osc[c, pl.ds(0, R // 2, stride=2), :].reshape(G2, 1, 8, 128)
            od = osc[c, pl.ds(1, R // 2, stride=2), :].reshape(G2, 1, 8, 128)
            on = jnp.concatenate([ev, od], axis=1).reshape(R, 128)
            o_sc[:, c * 128:(c + 1) * 128] = (on * linv).astype(_bf16)

    def pv(i, par, lo, hi):
        o = jnp.dot(pltpu.bitcast(ps[par][:, lo * 128:hi * 128], _bf16),
                    vbuf[slot(i), lo * 128:hi * 128, :], preferred_element_type=_f32)
        if lo > 0:
            o = o + opart[...]
        if hi < NC:
            opart[...] = o
        else:
            finish_o(o, par)

    def pv_exp(i, par, nch):
        pe = 1 - par
        mb = ms[pe][...]
        lacc = jnp.zeros((R, 128), _f32)
        cpc = NC // nch
        o = None
        for kc in range(nch):
            oc = jnp.dot(pltpu.bitcast(ps[par][:, kc * cpc * 128:(kc + 1) * cpc * 128], _bf16),
                         vbuf[slot(i), kc * cpc * 128:(kc + 1) * cpc * 128, :],
                         preferred_element_type=_f32)
            o = oc if o is None else o + oc
            for c in range(kc * cpc, (kc + 1) * cpc):
                lacc = exp_chunk(pe, mb, c, lacc, oc[:, (c % 2) * 128:(c % 2 + 1) * 128])
        ls[pe][...] = jnp.broadcast_to(jnp.sum(lacc, axis=1, keepdims=True), (R, 128))
        finish_o(o, par)

    def qk_exp(iq, parq, do_exp, lo, hi):
        pe = 1 - parq
        sn = lax.dot_general(q_all[iq], kbuf[slot(iq), lo * 128:hi * 128, :], _NT,
                             preferred_element_type=_f32)
        ss[parq][:, lo * 128:hi * 128] = sn
        if do_exp:
            mb = ms[pe][...]
        mx = sn[:, 0:128]
        for c in range(1, hi - lo):
            mx = jnp.maximum(mx, sn[:, c * 128:(c + 1) * 128])
        if lo > 0:
            mx = jnp.maximum(mx, mtmp[...])
        if hi < NC:
            mtmp[...] = mx
        else:
            ms[parq][...] = jnp.broadcast_to(jnp.max(mx, axis=1, keepdims=True), (R, 128))
        if do_exp:
            lacc = ltmp[...] if lo > 0 else jnp.zeros((R, 128), _f32)
            for c in range(lo, hi):
                lacc = exp_chunk(pe, mb, c, lacc, sn[:, (c - lo) * 128:(c - lo + 1) * 128])
            if hi < NC:
                ltmp[...] = lacc
            else:
                ls[pe][...] = jnp.broadcast_to(jnp.sum(lacc, axis=1, keepdims=True), (R, 128))

    def convert_out(b):
        out_sc[b] = acc_sc[b].astype(out_sc.dtype)

    x_copy.start()
    for h in range(Hkv):
        wq_copy(h).start()
    acc_sc[...] = jnp.zeros_like(acc_sc)
    x_copy.wait()

    def qbody(h, carry):
        wq_copy(h).wait()
        xa = x_sc[...].reshape(B * Sq, x_sc.shape[-1])
        q = jnp.dot(xa, wq_sc[h], preferred_element_type=_f32)
        q = (q * (Dh ** -0.5 * _LOG2E)).astype(_bf16)
        for b in range(B):
            for r in range(rep):
                q_all[h * B + b, r * Sq:(r + 1) * Sq, :] = q[b * Sq:(b + 1) * Sq, r * Dh:(r + 1) * Dh]

        @pl.when(h == 0)
        def _():
            k_copy(0).start()
            k_copy(1).start()
            k_copy(2).start()
            v_copy(0).start()
            wo_copy.start()
            for j in range(3, NB):
                k_copy(j).start()
                v_copy(j - 2).start()
            for j in range(NB - 2, NB):
                v_copy(j).start()
        return carry

    lax.fori_loop(0, Hkv, qbody, 0)

    k_copy(0).wait()
    qk_exp(0, 0, False, 0, NC)
    k_copy(NB).start()
    k_copy(1).wait()
    qk_exp(1, 1, True, 0, NC)
    k_copy(NB + 1).start()
    wo_copy.wait()

    def part(i, par, lo, hi):
        pv(i - 1, 1 - par, lo, hi)
        qk_exp(i + 1, 1 - par, True, lo, hi)
        if hi == NC:
            outproj(i - 1)

    def by_parity(i, lo, hi):
        odd = jnp.bitwise_and(i, 1)

        @pl.when(odd == 0)
        def _():
            part(i, 0, lo, hi)

        @pl.when(odd == 1)
        def _():
            part(i, 1, lo, hi)

    def starts(i):
        @pl.when(i + NB <= E)
        def _():
            k_copy(i + 1 + NB).start()
            v_copy(i - 1 + NB).start()

        @pl.when(jnp.logical_and(i + NB > E, i + NB <= N - 2))
        def _():
            for hf in range(2):
                k_copy(i + 1 + NB, hf).start()
                v_copy(i - 1 + NB, hf).start()

        @pl.when(jnp.logical_and(i + NB > N - 2, i - 1 + NB < N))
        def _():
            v_copy(i - 1 + NB).start()

    def body_full(i, carry):
        k_copy(i + 1).wait()
        v_copy(i - 1).wait()
        by_parity(i, 0, NC)
        starts(i)
        return carry

    def body_half(i, carry):
        k_copy(i + 1, 0).wait()
        v_copy(i - 1, 0).wait()
        by_parity(i, 0, NC // 2)
        k_copy(i + 1, 1).wait()
        v_copy(i - 1, 1).wait()
        by_parity(i, NC // 2, NC)
        starts(i)
        return carry

    lax.fori_loop(1, E + 1, body_full, 0)
    lax.fori_loop(E + 1, N - 1, body_half, 0)

    i = N - 1
    v_copy(i - 1).wait()
    pv_exp(i - 1, (i - 1) % 2, 4)
    outproj(i - 1)
    for b in range(B - 1):
        convert_out(b)
    v_copy(i).wait()
    for b in range(B - 1):
        out_copy(b).start()
    pv(i, i % 2, 0, NC)
    outproj(i)
    convert_out(B - 1)
    out_copy(B - 1).start()
    for b in range(B):
        out_copy(b).wait()


@jax.jit
def pallas_standalone__gqa_block_cached__near_ridge_kernel(
    x: jax.Array,
    k_cache: jax.Array,
    v_cache: jax.Array,
    wq: jax.Array,
    wo: jax.Array,
):
    B, Sq, D = x.shape
    _, Hkv, Sk, Dh = k_cache.shape
    Hq = wq.shape[1] // Dh
    rep = Hq // Hkv
    G = rep * Dh
    R = rep * Sq
    N = B * Hkv
    NB = 6
    E = N - 14
    assert B & (B - 1) == 0 and R % 16 == 0 and Sk % 512 == 0 and Dh == 256
    assert 3 <= NB <= E <= N - 2

    kern = functools.partial(_kernel, B=B, Sq=Sq, Dh=Dh, rep=rep, Hkv=Hkv, Sk=Sk, NB=NB, E=E)
    hbm = pl.BlockSpec(memory_space=pl.ANY)
    stat = pltpu.VMEM((R, 128), _f32)
    return pl.pallas_call(
        kern,
        in_specs=[hbm] * 5,
        out_specs=hbm,
        out_shape=jax.ShapeDtypeStruct((B, Sq, D), x.dtype),
        scratch_shapes=[
            pltpu.VMEM((B, Sq, D), _bf16),
            pltpu.VMEM((Hkv, D, G), _bf16),
            pltpu.VMEM((D, Hq * Dh), _bf16),
            pltpu.VMEM((NB, Sk, Dh), _bf16),
            pltpu.VMEM((NB, Sk, Dh), _bf16),
            pltpu.VMEM((N, R, Dh), _bf16),
            pltpu.VMEM((R, Dh), _bf16),
            pltpu.VMEM((B, Sq, D), _f32),
            pltpu.VMEM((R, Sk), _f32), pltpu.VMEM((R, Sk), _f32),
            stat, stat,
            pltpu.VMEM((R // 2, Sk), jnp.uint32), pltpu.VMEM((R // 2, Sk), jnp.uint32),
            stat, stat,
            pltpu.VMEM((Dh // 128, R, 128), _f32),
            pltpu.VMEM((R, Dh), _f32),
            stat, stat,
            pltpu.VMEM((B, Sq, D), x.dtype),
            pltpu.SemaphoreType.DMA((2, NB)),
            pltpu.SemaphoreType.DMA((2, NB)),
            pltpu.SemaphoreType.DMA((2,)),
            pltpu.SemaphoreType.DMA((Hkv,)),
            pltpu.SemaphoreType.DMA((B,)),
        ],
        compiler_params=pltpu.CompilerParams(
            vmem_limit_bytes=100 * 1024 * 1024,
            disable_bounds_checks=True,
        ),
    )(x, k_cache, v_cache, wq, wo.T)
```

```python
import functools

import jax
import jax.numpy as jnp
from jax import lax
import jax.experimental.pallas as pl
import jax.experimental.pallas.tpu as pltpu

_NT = (((1,), (1,)), ((), ()))
_f32, _bf16 = jnp.float32, jnp.bfloat16


def _kernel(x_hbm, k_hbm, v_hbm, wq_hbm, wot_hbm, out_hbm,
            x_sc, wq_sc, wo_sc, kbuf, vbuf, q_all, o_sc, acc_sc,
            s0, s1, m0, m1, p0, p1, l0, l1,
            opart, mtmp, ltmp, out_sc,
            sem_k, sem_v, sem_w, sem_q, sem_o,
            *, B, Sq, Dh, rep, Hkv, Sk, NB, E):
    N = B * Hkv
    G = rep * Dh
    R = rep * Sq
    NC = Sk // 128
    HS = Sk // 2
    LB = B.bit_length() - 1
    ss, ms, ps, ls = (s0, s1), (m0, m1), (p0, p1), (l0, l1)

    def slot(i):
        return i % NB if isinstance(i, int) else lax.rem(i, NB)

    def bidx(i):
        return i % B if isinstance(i, int) else jnp.bitwise_and(i, B - 1)

    def hidx(i):
        return i // B if isinstance(i, int) else lax.shift_right_logical(i, LB)

    def kv_copy(hbm, buf, sem, i, hf):
        if hf is None:
            return pltpu.make_async_copy(hbm.at[bidx(i), hidx(i)], buf.at[slot(i)], sem.at[0, slot(i)])
        return pltpu.make_async_copy(hbm.at[bidx(i), hidx(i), pl.ds(hf * HS, HS)],
                                     buf.at[slot(i), pl.ds(hf * HS, HS)], sem.at[hf, slot(i)])

    def k_copy(i, hf=None):
        return kv_copy(k_hbm, kbuf, sem_k, i, hf)

    def v_copy(i, hf=None):
        return kv_copy(v_hbm, vbuf, sem_v, i, hf)

    x_copy = pltpu.make_async_copy(x_hbm, x_sc, sem_w.at[0])
    wo_copy = pltpu.make_async_copy(wot_hbm, wo_sc, sem_w.at[1])

    def wq_copy(h):
        col = h * G if isinstance(h, int) else pl.multiple_of(h * G, G)
        return pltpu.make_async_copy(wq_hbm.at[:, pl.ds(col, G)], wq_sc.at[h], sem_q.at[h])

    def out_copy(b):
        return pltpu.make_async_copy(out_sc.at[b], out_hbm.at[b], sem_o.at[b])

    def outproj(i):
        h = hidx(i)
        b = bidx(i)
        part = acc_sc[b]
        for r in range(rep):
            col = pl.multiple_of(h * G + r * Dh, Dh)
            part = part + lax.dot_general(o_sc[r * Sq:(r + 1) * Sq, :], wo_sc[:, pl.ds(col, Dh)], _NT,
                                          preferred_element_type=_f32)
        acc_sc[b] = part

    def exp_chunk(pe, mb, c, lacc, pace):
        xx = ss[pe][:, c * 128:(c + 1) * 128] - mb
        xx = jnp.minimum(xx, jnp.abs(pace))
        p = jnp.exp(xx)
        ps[pe][:, c * 128:(c + 1) * 128] = p.astype(_bf16)
        return lacc + p

    def finish_o(o, par):
        linv = 1.0 / ls[par][...]
        for c in range(Dh // 128):
            o_sc[:, c * 128:(c + 1) * 128] = (o[:, c * 128:(c + 1) * 128] * linv).astype(_bf16)

    def pv(i, par, lo, hi):
        o = jnp.dot(ps[par][:, lo * 128:hi * 128],
                    vbuf[slot(i), lo * 128:hi * 128, :], preferred_element_type=_f32)
        if lo > 0:
            o = o + opart[...]
        if hi < NC:
            opart[...] = o
        else:
            finish_o(o, par)

    def pv_exp(i, par, nch):
        pe = 1 - par
        mb = ms[pe][...]
        lacc = jnp.zeros((R, 128), _f32)
        cpc = NC // nch
        o = None
        for kc in range(nch):
            oc = jnp.dot(ps[par][:, kc * cpc * 128:(kc + 1) * cpc * 128],
                         vbuf[slot(i), kc * cpc * 128:(kc + 1) * cpc * 128, :],
                         preferred_element_type=_f32)
            o = oc if o is None else o + oc
            for c in range(kc * cpc, (kc + 1) * cpc):
                lacc = exp_chunk(pe, mb, c, lacc, oc[:, (c % 2) * 128:(c % 2 + 1) * 128])
        ls[pe][...] = jnp.broadcast_to(jnp.sum(lacc, axis=1, keepdims=True), (R, 128))
        finish_o(o, par)

    def qk_exp(iq, parq, do_exp, lo, hi):
        pe = 1 - parq
        sn = lax.dot_general(q_all[iq], kbuf[slot(iq), lo * 128:hi * 128, :], _NT,
                             preferred_element_type=_f32)
        ss[parq][:, lo * 128:hi * 128] = sn
        if do_exp:
            mb = ms[pe][...]
        mx = sn[:, 0:128]
        for c in range(1, hi - lo):
            mx = jnp.maximum(mx, sn[:, c * 128:(c + 1) * 128])
        if lo > 0:
            mx = jnp.maximum(mx, mtmp[...])
        if hi < NC:
            mtmp[...] = mx
        else:
            ms[parq][...] = jnp.broadcast_to(jnp.max(mx, axis=1, keepdims=True), (R, 128))
        if do_exp:
            lacc = ltmp[...] if lo > 0 else jnp.zeros((R, 128), _f32)
            for c in range(lo, hi):
                lacc = exp_chunk(pe, mb, c, lacc, sn[:, (c - lo) * 128:(c - lo + 1) * 128])
            if hi < NC:
                ltmp[...] = lacc
            else:
                ls[pe][...] = jnp.broadcast_to(jnp.sum(lacc, axis=1, keepdims=True), (R, 128))

    def convert_out(b):
        out_sc[b] = acc_sc[b].astype(out_sc.dtype)

    x_copy.start()
    for h in range(Hkv):
        wq_copy(h).start()
    acc_sc[...] = jnp.zeros_like(acc_sc)
    x_copy.wait()

    def qbody(h, carry):
        wq_copy(h).wait()
        xa = x_sc[...].reshape(B * Sq, x_sc.shape[-1])
        q = jnp.dot(xa, wq_sc[h], preferred_element_type=_f32)
        q = (q * (Dh ** -0.5)).astype(_bf16)
        for b in range(B):
            for r in range(rep):
                q_all[h * B + b, r * Sq:(r + 1) * Sq, :] = q[b * Sq:(b + 1) * Sq, r * Dh:(r + 1) * Dh]

        @pl.when(h == 0)
        def _():
            k_copy(0).start()
            k_copy(1).start()
            k_copy(2).start()
            v_copy(0).start()
            wo_copy.start()
            for j in range(3, NB):
                k_copy(j).start()
                v_copy(j - 2).start()
            for j in range(NB - 2, NB):
                v_copy(j).start()
        return carry

    lax.fori_loop(0, Hkv, qbody, 0)

    k_copy(0).wait()
    qk_exp(0, 0, False, 0, NC)
    k_copy(NB).start()
    k_copy(1).wait()
    qk_exp(1, 1, True, 0, NC)
    k_copy(NB + 1).start()
    wo_copy.wait()

    def part(i, par, lo, hi):
        pv(i - 1, 1 - par, lo, hi)
        qk_exp(i + 1, 1 - par, True, lo, hi)
        if hi == NC:
            outproj(i - 1)

    def by_parity(i, lo, hi):
        odd = jnp.bitwise_and(i, 1)

        @pl.when(odd == 0)
        def _():
            part(i, 0, lo, hi)

        @pl.when(odd == 1)
        def _():
            part(i, 1, lo, hi)

    def starts(i):
        @pl.when(i + NB <= E)
        def _():
            k_copy(i + 1 + NB).start()
            v_copy(i - 1 + NB).start()

        @pl.when(jnp.logical_and(i + NB > E, i + NB <= N - 2))
        def _():
            for hf in range(2):
                k_copy(i + 1 + NB, hf).start()
                v_copy(i - 1 + NB, hf).start()

        @pl.when(jnp.logical_and(i + NB > N - 2, i - 1 + NB < N))
        def _():
            v_copy(i - 1 + NB).start()

    def body_full(i, carry):
        k_copy(i + 1).wait()
        v_copy(i - 1).wait()
        by_parity(i, 0, NC)
        starts(i)
        return carry

    def body_half(i, carry):
        k_copy(i + 1, 0).wait()
        v_copy(i - 1, 0).wait()
        by_parity(i, 0, NC // 2)
        k_copy(i + 1, 1).wait()
        v_copy(i - 1, 1).wait()
        by_parity(i, NC // 2, NC)
        starts(i)
        return carry

    lax.fori_loop(1, E + 1, body_full, 0)
    lax.fori_loop(E + 1, N - 1, body_half, 0)

    i = N - 1
    v_copy(i - 1).wait()
    pv_exp(i - 1, (i - 1) % 2, 4)
    outproj(i - 1)
    for b in range(B - 1):
        convert_out(b)
    v_copy(i).wait()
    for b in range(B - 1):
        out_copy(b).start()
    pv(i, i % 2, 0, NC)
    outproj(i)
    convert_out(B - 1)
    out_copy(B - 1).start()
    for b in range(B):
        out_copy(b).wait()


@jax.jit
def pallas_standalone__gqa_block_cached__near_ridge_kernel(
    x: jax.Array,
    k_cache: jax.Array,
    v_cache: jax.Array,
    wq: jax.Array,
    wo: jax.Array,
):
    B, Sq, D = x.shape
    _, Hkv, Sk, Dh = k_cache.shape
    Hq = wq.shape[1] // Dh
    rep = Hq // Hkv
    G = rep * Dh
    R = rep * Sq
    N = B * Hkv
    NB = 6
    E = N - 14
    assert B & (B - 1) == 0 and R % 16 == 0 and Sk % 512 == 0 and Dh == 256
    assert 3 <= NB <= E <= N - 2

    kern = functools.partial(_kernel, B=B, Sq=Sq, Dh=Dh, rep=rep, Hkv=Hkv, Sk=Sk, NB=NB, E=E)
    hbm = pl.BlockSpec(memory_space=pl.ANY)
    stat = pltpu.VMEM((R, 128), _f32)
    return pl.pallas_call(
        kern,
        in_specs=[hbm] * 5,
        out_specs=hbm,
        out_shape=jax.ShapeDtypeStruct((B, Sq, D), x.dtype),
        scratch_shapes=[
            pltpu.VMEM((B, Sq, D), _bf16),
            pltpu.VMEM((Hkv, D, G), _bf16),
            pltpu.VMEM((D, Hq * Dh), _bf16),
            pltpu.VMEM((NB, Sk, Dh), _bf16),
            pltpu.VMEM((NB, Sk, Dh), _bf16),
            pltpu.VMEM((N, R, Dh), _bf16),
            pltpu.VMEM((R, Dh), _bf16),
            pltpu.VMEM((B, Sq, D), _f32),
            pltpu.VMEM((R, Sk), _f32), pltpu.VMEM((R, Sk), _f32),
            stat, stat,
            pltpu.VMEM((R, Sk), _bf16), pltpu.VMEM((R, Sk), _bf16),
            stat, stat,
            pltpu.VMEM((R, Dh), _f32),
            stat, stat,
            pltpu.VMEM((B, Sq, D), x.dtype),
            pltpu.SemaphoreType.DMA((2, NB)),
            pltpu.SemaphoreType.DMA((2, NB)),
            pltpu.SemaphoreType.DMA((2,)),
            pltpu.SemaphoreType.DMA((Hkv,)),
            pltpu.SemaphoreType.DMA((B,)),
        ],
        compiler_params=pltpu.CompilerParams(
            vmem_limit_bytes=64 * 1024 * 1024,
            disable_bounds_checks=True,
        ),
    )(x, k_cache, v_cache, wq, wo.T)
```
